```python
import jax
import jax.numpy as jnp

def _softmax(x, axis=-1):
    return jax.nn.softmax(x, axis=axis)
def _gelu(x):
    return jax.nn.gelu(x, approximate=True)
def _silu(x):
    return jax.nn.silu(x)
def _sigmoid(x):
    return jax.nn.sigmoid(x)
def _layernorm(x, axis=-1, eps=1e-5):
    m = jnp.mean(x, axis=axis, keepdims=True)
    v = jnp.var(x, axis=axis, keepdims=True)
    return (x - m) / jnp.sqrt(v + eps)
def _scatter_add(tgt, idx, src, axis=0):
    return tgt.at[idx].add(src)
def _segment_sum(src, seg, n):
    return jax.ops.segment_sum(src, seg, n)
class _Rng:
    def __init__(self, key):
        self._k = key
    def _next(self):
        self._k, sub = jax.random.split(self._k)
        return sub
    def normal(self, shape):
        return jax.random.normal(self._next(), shape, dtype=jnp.bfloat16)
    def randint(self, lo, hi, shape):
        return jax.random.randint(self._next(), shape, lo, hi, dtype=jnp.int32)
    def uniform(self, shape, lo=0.0, hi=1.0):
        return jax.random.uniform(self._next(), shape, jnp.bfloat16, lo, hi)
    def permutation(self, n):
        return jax.random.permutation(self._next(), n)


kernel_name = 'recurrent_scan__sliding_block_cached__glu_gated_glu__decode'

def setup_inputs():
    _rng = _Rng(jax.random.key(int.from_bytes(__import__("os").urandom(4), "little")))
    _w = (lambda a: (lambda t: t.astype(jnp.bfloat16) if jnp.issubdtype(t.dtype, jnp.floating) else t)(jnp.asarray(a)))
    def _A_setup():
        B, Sq, D = 1, 1, 576
        Hq, Hkv, Sk, Dh = 32, 16, 65536, 128
        assert Hq % Hkv == 0, (Hq, Hkv)
        return {
            "x": _w((lambda *s: _rng.normal(s) * 0.05)(B, Sq, D)),
            "k_cache": _w((lambda *s: _rng.normal(s) * 0.05)(B, Hkv, Sk, Dh)),
            "v_cache": _w((lambda *s: _rng.normal(s) * 0.05)(B, Hkv, Sk, Dh)),
            "wq": _w((lambda *s: _rng.normal(s) * 0.05)(D, Hq * Dh) * (D ** -0.5)),
            "wo": _w((lambda *s: _rng.normal(s) * 0.05)(Hq * Dh, D) * ((Hq * Dh) ** -0.5)),
        }
    _A_in = _A_setup()

    def _B_setup():
        B, S, D, F = 1, 1, 576, 4608
        return {
            "x": _w((lambda *s: _rng.normal(s) * 0.05)(B, S, D)),
            "w_gate": _w((lambda *s: _rng.normal(s) * 0.05)(D, F)),
            "w_up": _w((lambda *s: _rng.normal(s) * 0.05)(D, F)),
            "w_down": _w((lambda *s: _rng.normal(s) * 0.05)(F, D)),
        }
    _B_in = _B_setup()

    return {
        "A_x": _A_in["x"],
        "A_k_cache": _A_in["k_cache"],
        "A_v_cache": _A_in["v_cache"],
        "A_wq": _A_in["wq"],
        "A_wo": _A_in["wo"],
        "B_x": _B_in["x"],
        "B_w_gate": _B_in["w_gate"],
        "B_w_up": _B_in["w_up"],
        "B_w_down": _B_in["w_down"],
    }

def reference(A_x, A_k_cache, A_v_cache, A_wq, A_wo, B_x, B_w_gate, B_w_up, B_w_down):
    def _A_ref(x, k_cache, v_cache, wq, wo):
        B, Sq, D = x.shape
        Hq, Dh = 32, 128
        Hkv, Sk = k_cache.shape[1], k_cache.shape[2]
        W = min(4096, max(256, Sk // 4))
        rep = Hq // Hkv
        q = (lambda x, *d: x.transpose(*d))((x @ wq).reshape(B, Sq, Hq, Dh), 0, 2, 1, 3)
        k = jnp.repeat(k_cache[:, :, Sk - W:, :], rep, axis=1)
        v = jnp.repeat(v_cache[:, :, Sk - W:, :], rep, axis=1)
        scores = jnp.einsum("bhqd,bhkd->bhqk", q, k) * (Dh ** -0.5)
        p = _softmax(scores, axis=-1)
        o = jnp.einsum("bhqk,bhkd->bhqd", p, v)
        return (lambda x, *d: x.transpose(*d))(o, 0, 2, 1, 3).reshape(B, Sq, Hq * Dh) @ wo

    def _B_ref(x, w_gate, w_up, w_down):
        g = jnp.einsum("bsd,df->bsf", x, w_gate)
        u = jnp.einsum("bsd,df->bsf", x, w_up)
        h = _sigmoid(g) * u
        return jnp.einsum("bsf,fd->bsd", h, w_down)

    x = A_x
    xn = _layernorm(x, axis=-1)
    s = _A_ref(xn, A_k_cache, A_v_cache, A_wq, A_wo)
    g = _silu(_B_ref(xn, B_w_gate, B_w_up, B_w_down))
    return x + s * g
```

```python
import jax
import jax.numpy as jnp
from jax import lax
import jax.experimental.pallas as pl
import jax.experimental.pallas.tpu as pltpu

_NN = (((1,), (0,)), ((), ()))
_NT = (((1,), (1,)), ((), ()))
_HQ, _DH = 32, 128
_ROWS = 8
_DOWN_SPLIT = (3328, 896, 256, 128)


def _dot(a, b, dims):
    return lax.dot_general(a, b, dims, preferred_element_type=jnp.float32)


def _chunk(i, size):
    return pl.ds(pl.multiple_of(i * size, size), size)


def _kernel(x_hbm, k_hbm, v_hbm, wq_hbm, wo_hbm, wg_hbm, wu_hbm, wd_hbm, o_ref,
            x_v, wq_v, k_v, v_v, wo_v, wg_v, wu_v, wd_v,
            q_s, p_s, l_s, o_s, h_s, acc_s, last_sem):
    f32, bf16 = jnp.float32, jnp.bfloat16
    d_model, ffn = wg_hbm.shape
    hkv, sk = k_hbm.shape[1], k_hbm.shape[2]
    win = k_v.shape[1]
    hd = _HQ * _DH

    def down_copy(lo, n, sem):
        return pltpu.make_async_copy(wd_hbm.at[:, pl.ds(lo, n)], wd_v.at[:, pl.ds(lo, n)], sem)

    def down_dot(cols):
        return _dot(h_s[:, cols].astype(bf16), wd_v[:, cols], _NT)

    last_n = _DOWN_SPLIT[-1]
    last_lo = ffn - last_n
    c_last = down_copy(last_lo, last_n, last_sem)

    def main(sems):
        window = pl.ds(sk - win, win)
        c_wq = pltpu.make_async_copy(wq_hbm, wq_v, sems.at[0])
        c_x = pltpu.make_async_copy(x_hbm, x_v, sems.at[1])
        c_wg = pltpu.make_async_copy(wg_hbm, wg_v, sems.at[2])
        c_wu = pltpu.make_async_copy(wu_hbm, wu_v, sems.at[2])
        c_k = pltpu.make_async_copy(k_hbm.at[0, :, window, :], k_v, sems.at[3])
        c_v = pltpu.make_async_copy(v_hbm.at[0, :, window, :], v_v, sems.at[4])
        c_wo = pltpu.make_async_copy(wo_hbm, wo_v, sems.at[5])
        c_wd, lo = [], 0
        for j, n in enumerate(_DOWN_SPLIT[:-1]):
            c_wd.append((lo, n, down_copy(lo, n, sems.at[6 + j])))
            lo += n
        for c in [c_wq, c_x, c_wg, c_wu, c_k, c_v, c_wo] + [c for _, _, c in c_wd] + [c_last]:
            c.start()

        c_x.wait()
        x = x_v[...].astype(f32)
        xc = x - jnp.mean(x, axis=-1, keepdims=True)
        var = jnp.mean(xc * xc, axis=-1, keepdims=True)
        xn = jnp.broadcast_to(xc / jnp.sqrt(var + 1e-5), (_ROWS, d_model)).astype(bf16)

        c_wq.wait()

        @pl.loop(0, hd // 512)
        def _(i):
            q_s[:, _chunk(i, 512)] = _dot(xn, wq_v[:, _chunk(i, 512)], _NN)

        c_wg.wait()
        c_wu.wait()

        @pl.loop(0, ffn // 512)
        def _(i):
            g = _dot(xn, wg_v[:, _chunk(i, 512)], _NN)
            u = _dot(xn, wu_v[:, _chunk(i, 512)], _NN)
            h_s[:, _chunk(i, 512)] = jax.nn.sigmoid(g) * u

        c_k.wait()

        @pl.loop(0, hkv)
        def _(h):
            qq = q_s[:, _chunk(h, 2 * _DH)]
            row = lax.broadcasted_iota(jnp.int32, (_ROWS, _DH), 0)
            q2 = jnp.where(row == 0, qq[:, :_DH], qq[:, _DH:]).astype(bf16)
            s = _dot(q2, k_v[h], _NT) * (_DH ** -0.5)
            e = jnp.exp(s - jnp.max(s, axis=-1, keepdims=True))
            p_s[h] = e
            l_s[h] = jnp.broadcast_to(jnp.sum(e, axis=-1, keepdims=True), (_ROWS, _DH))

        c_v.wait()

        @pl.loop(0, hkv)
        def _(h):
            o = _dot(p_s[h].astype(bf16), v_v[h], _NN) / l_s[h]
            o_s[:, _chunk(h, 2 * _DH)] = jnp.concatenate(
                [jnp.broadcast_to(o[0:1], (_ROWS, _DH)), jnp.broadcast_to(o[1:2], (_ROWS, _DH))], axis=1)

        c_wo.wait()
        acc_s[0] = lax.fori_loop(
            0, hd // 1024,
            lambda i, acc: acc + _dot(o_s[:, _chunk(i, 1024)].astype(bf16), wo_v[:, _chunk(i, 1024)], _NT),
            jnp.zeros((_ROWS, d_model), f32))

        b = jnp.zeros((_ROWS, d_model), f32)
        step = 1152
        for lo, n, c in c_wd:
            c.wait()
            if n // step >= 2:
                b = lax.fori_loop(
                    0, n // step,
                    lambda i, acc, lo=lo: acc + down_dot(pl.ds(pl.multiple_of(lo + i * step, 128), step)), b)
                lo, n = lo + n // step * step, n % step
            if n:
                b = b + down_dot(pl.ds(lo, n))
        acc_s[1] = b

    pl.run_scoped(main, pltpu.SemaphoreType.DMA((5 + len(_DOWN_SPLIT),)))
    c_last.wait()
    b = acc_s[1] + down_dot(pl.ds(last_lo, last_n))
    out = x_v[...].astype(f32) + (acc_s[0] * (b * jax.nn.sigmoid(b)))[0:1]
    o_ref[...] = out.astype(o_ref.dtype)


@jax.jit
def pallas_recurrent_scan__sliding_block_cached__glu_gated_glu__decode_kernel(
    A_x: jax.Array,
    A_k_cache: jax.Array,
    A_v_cache: jax.Array,
    A_wq: jax.Array,
    A_wo: jax.Array,
    B_x: jax.Array,
    B_w_gate: jax.Array,
    B_w_up: jax.Array,
    B_w_down: jax.Array,
):
    del B_x
    batch, seq, d_model = A_x.shape
    _, hkv, sk, dh = A_k_cache.shape
    ffn = B_w_gate.shape[1]
    hd = _HQ * _DH
    win = min(4096, max(256, sk // 4))
    assert (batch, seq, dh) == (1, 1, _DH) and _HQ == 2 * hkv and ffn == sum(_DOWN_SPLIT)
    f32 = jnp.float32
    out = pl.pallas_call(
        _kernel,
        out_shape=jax.ShapeDtypeStruct((1, d_model), A_x.dtype),
        in_specs=[pl.BlockSpec(memory_space=pl.ANY)] * 8,
        out_specs=pl.BlockSpec(memory_space=pltpu.VMEM),
        scratch_shapes=[
            pltpu.VMEM((1, d_model), A_x.dtype),
            pltpu.VMEM((d_model, hd), A_wq.dtype),
            pltpu.VMEM((hkv, win, dh), A_k_cache.dtype),
            pltpu.VMEM((hkv, win, dh), A_v_cache.dtype),
            pltpu.VMEM((d_model, hd), A_wo.dtype),
            pltpu.VMEM((d_model, ffn), B_w_gate.dtype),
            pltpu.VMEM((d_model, ffn), B_w_up.dtype),
            pltpu.VMEM((d_model, ffn), B_w_down.dtype),
            pltpu.VMEM((_ROWS, hd), f32),
            pltpu.VMEM((hkv, _ROWS, win), f32),
            pltpu.VMEM((hkv, _ROWS, dh), f32),
            pltpu.VMEM((_ROWS, hd), f32),
            pltpu.VMEM((_ROWS, ffn), f32),
            pltpu.VMEM((2, _ROWS, d_model), f32),
            pltpu.SemaphoreType.DMA(()),
        ],
        compiler_params=pltpu.CompilerParams(vmem_limit_bytes=100 * 1024 * 1024),
    )(
        A_x.reshape(1, d_model), A_k_cache, A_v_cache, A_wq,
        A_wo.T, B_w_gate, B_w_up, B_w_down.T,
    )
    return out.reshape(batch, seq, d_model)
```

```python
import jax
import jax.numpy as jnp
from jax import lax
import jax.experimental.pallas as pl
import jax.experimental.pallas.tpu as pltpu

_NN = (((1,), (0,)), ((), ()))
_NT = (((1,), (1,)), ((), ()))
_HQ, _DH = 32, 128
_ROWS = 8
_DOWN_SPLIT = (3072, 1024, 256, 256)
_TAIL = 2


def _dot(a, b, dims):
    return lax.dot_general(a, b, dims, preferred_element_type=jnp.float32)


def _chunk(i, size):
    return pl.ds(pl.multiple_of(i * size, size), size)


def _kernel(x_hbm, k_hbm, v_hbm, wq_hbm, wo_hbm, wg_hbm, wu_hbm, wd_hbm, o_ref,
            x_v, wq_v, k_v, v_v, wo_v, wg_v, wu_v, wd_v,
            q_s, p_s, l_s, o_s, h_s, acc_s, tail_sems):
    f32, bf16 = jnp.float32, jnp.bfloat16
    d_model, ffn = wg_hbm.shape
    hkv, sk = k_hbm.shape[1], k_hbm.shape[2]
    win = k_v.shape[1]
    hd = _HQ * _DH

    def down_pieces(first, count, sems, sem0):
        pieces = []
        for j in range(count):
            cols = pl.ds(sum(_DOWN_SPLIT[:first + j]), _DOWN_SPLIT[first + j])
            pieces.append((cols, pltpu.make_async_copy(wd_hbm.at[:, cols], wd_v.at[:, cols], sems.at[sem0 + j])))
        return pieces

    def down_dot(cols):
        return _dot(h_s[:, cols].astype(bf16), wd_v[:, cols], _NT)

    def consume_down(pieces, b):
        for cols, copy in pieces:
            copy.wait()
            if cols.size > 1024:
                b = lax.fori_loop(cols.start // 1024, (cols.start + cols.size) // 1024,
                                  lambda i, acc: acc + down_dot(_chunk(i, 1024)), b)
            else:
                b = b + down_dot(cols)
        return b

    n_body = len(_DOWN_SPLIT) - _TAIL
    tail = down_pieces(n_body, _TAIL, tail_sems, 0)

    def main(sems):
        window = pl.ds(sk - win, win)
        c_wq = pltpu.make_async_copy(wq_hbm, wq_v, sems.at[0])
        c_x = pltpu.make_async_copy(x_hbm, x_v, sems.at[1])
        c_wg = pltpu.make_async_copy(wg_hbm, wg_v, sems.at[2])
        c_wu = pltpu.make_async_copy(wu_hbm, wu_v, sems.at[2])
        c_k = pltpu.make_async_copy(k_hbm.at[0, :, window, :], k_v, sems.at[3])
        c_v = pltpu.make_async_copy(v_hbm.at[0, :, window, :], v_v, sems.at[4])
        c_wo = pltpu.make_async_copy(wo_hbm, wo_v, sems.at[5])
        body = down_pieces(0, n_body, sems, 6)
        for c in [c_wq, c_x, c_wg, c_wu, c_k, c_v, c_wo] + [c for _, c in body + tail]:
            c.start()

        c_x.wait()
        x = x_v[...].astype(f32)
        xc = x - jnp.mean(x, axis=-1, keepdims=True)
        var = jnp.mean(xc * xc, axis=-1, keepdims=True)
        xn = jnp.broadcast_to(xc / jnp.sqrt(var + 1e-5), (_ROWS, d_model)).astype(bf16)

        c_wq.wait()

        @pl.loop(0, hd // 512)
        def _(i):
            q_s[:, _chunk(i, 512)] = _dot(xn, wq_v[:, _chunk(i, 512)], _NN)

        c_wg.wait()
        c_wu.wait()

        @pl.loop(0, ffn // 512)
        def _(i):
            g = _dot(xn, wg_v[:, _chunk(i, 512)], _NN)
            u = _dot(xn, wu_v[:, _chunk(i, 512)], _NN)
            h_s[:, _chunk(i, 512)] = jax.nn.sigmoid(g) * u

        c_k.wait()

        @pl.loop(0, hkv)
        def _(h):
            qq = q_s[:, _chunk(h, 2 * _DH)]
            row = lax.broadcasted_iota(jnp.int32, (_ROWS, _DH), 0)
            q2 = jnp.where(row == 0, qq[:, :_DH], qq[:, _DH:]).astype(bf16)
            s = _dot(q2, k_v[h], _NT) * (_DH ** -0.5)
            e = jnp.exp(s - jnp.max(s, axis=-1, keepdims=True))
            p_s[h] = e
            l_s[h] = jnp.broadcast_to(jnp.sum(e, axis=-1, keepdims=True), (_ROWS, _DH))

        c_v.wait()

        @pl.loop(0, hkv)
        def _(h):
            o = _dot(p_s[h].astype(bf16), v_v[h], _NN) / l_s[h]
            o_s[:, _chunk(h, 2 * _DH)] = jnp.concatenate(
                [jnp.broadcast_to(o[0:1], (_ROWS, _DH)), jnp.broadcast_to(o[1:2], (_ROWS, _DH))], axis=1)

        c_wo.wait()
        acc_s[0] = lax.fori_loop(
            0, hd // 1024,
            lambda i, acc: acc + _dot(o_s[:, _chunk(i, 1024)].astype(bf16), wo_v[:, _chunk(i, 1024)], _NT),
            jnp.zeros((_ROWS, d_model), f32))

        acc_s[1] = consume_down(body, jnp.zeros((_ROWS, d_model), f32))

    pl.run_scoped(main, pltpu.SemaphoreType.DMA((6 + n_body,)))
    b = consume_down(tail, acc_s[1])
    out = x_v[...].astype(f32) + (acc_s[0] * (b * jax.nn.sigmoid(b)))[0:1]
    o_ref[...] = out.astype(o_ref.dtype)


@jax.jit
def pallas_recurrent_scan__sliding_block_cached__glu_gated_glu__decode_kernel(
    A_x: jax.Array,
    A_k_cache: jax.Array,
    A_v_cache: jax.Array,
    A_wq: jax.Array,
    A_wo: jax.Array,
    B_x: jax.Array,
    B_w_gate: jax.Array,
    B_w_up: jax.Array,
    B_w_down: jax.Array,
):
    del B_x
    batch, seq, d_model = A_x.shape
    _, hkv, sk, dh = A_k_cache.shape
    ffn = B_w_gate.shape[1]
    hd = _HQ * _DH
    win = min(4096, max(256, sk // 4))
    assert (batch, seq, dh) == (1, 1, _DH) and _HQ == 2 * hkv and ffn == sum(_DOWN_SPLIT)
    f32 = jnp.float32
    out = pl.pallas_call(
        _kernel,
        out_shape=jax.ShapeDtypeStruct((1, d_model), A_x.dtype),
        in_specs=[pl.BlockSpec(memory_space=pl.ANY)] * 8,
        out_specs=pl.BlockSpec(memory_space=pltpu.VMEM),
        scratch_shapes=[
            pltpu.VMEM((1, d_model), A_x.dtype),
            pltpu.VMEM((d_model, hd), A_wq.dtype),
            pltpu.VMEM((hkv, win, dh), A_k_cache.dtype),
            pltpu.VMEM((hkv, win, dh), A_v_cache.dtype),
            pltpu.VMEM((d_model, hd), A_wo.dtype),
            pltpu.VMEM((d_model, ffn), B_w_gate.dtype),
            pltpu.VMEM((d_model, ffn), B_w_up.dtype),
            pltpu.VMEM((d_model, ffn), B_w_down.dtype),
            pltpu.VMEM((_ROWS, hd), f32),
            pltpu.VMEM((hkv, _ROWS, win), f32),
            pltpu.VMEM((hkv, _ROWS, dh), f32),
            pltpu.VMEM((_ROWS, hd), f32),
            pltpu.VMEM((_ROWS, ffn), f32),
            pltpu.VMEM((2, _ROWS, d_model), f32),
            pltpu.SemaphoreType.DMA((_TAIL,)),
        ],
        compiler_params=pltpu.CompilerParams(vmem_limit_bytes=100 * 1024 * 1024),
    )(
        A_x.reshape(1, d_model), A_k_cache, A_v_cache, A_wq,
        A_wo.T, B_w_gate, B_w_up, B_w_down.T,
    )
    return out.reshape(batch, seq, d_model)
```
